```python
import os as _os
_os.environ.setdefault("JAX_PLATFORMS", "cpu")
import jax
import jax.numpy as jnp

def _softmax(x, axis=-1):
    return jax.nn.softmax(x, axis=axis)
def _gelu(x):
    return jax.nn.gelu(x, approximate=True)
def _silu(x):
    return jax.nn.silu(x)
def _sigmoid(x):
    return jax.nn.sigmoid(x)
def _layernorm(x, axis=-1, eps=1e-5):
    m = jnp.mean(x, axis=axis, keepdims=True)
    v = jnp.var(x, axis=axis, keepdims=True)
    return (x - m) / jnp.sqrt(v + eps)
def _scatter_add(tgt, idx, src, axis=0):
    return tgt.at[idx].add(src)
def _segment_sum(src, seg, n):
    return jax.ops.segment_sum(src, seg, n)
class _Rng:
    def __init__(self, key):
        self._k = key
    def _next(self):
        self._k, sub = jax.random.split(self._k)
        return sub
    def normal(self, shape):
        return jax.random.normal(self._next(), shape, dtype=jnp.bfloat16)
    def randint(self, lo, hi, shape):
        return jax.random.randint(self._next(), shape, lo, hi, dtype=jnp.int32)
    def uniform(self, shape, lo=0.0, hi=1.0):
        return jax.random.uniform(self._next(), shape, jnp.bfloat16, lo, hi)
    def permutation(self, n):
        return jax.random.permutation(self._next(), n)


kernel_name = 'concat_heads__gqa_block_cached__gqa_block_cached__near_ridge'

def setup_inputs():
    _rng = _Rng(jax.random.key(int.from_bytes(__import__("os").urandom(4), "little")))
    _w = (lambda a: (lambda t: t.astype(jnp.bfloat16) if jnp.issubdtype(t.dtype, jnp.floating) else t)(jnp.asarray(a)))
    def _A_setup():
        B, Sq, D = 8, 240, 640
        Hq, Hkv, Sk, Dh = 32, 32, 1024, 192
        assert Hq % Hkv == 0, (Hq, Hkv)
        return {
            "x": _w((lambda *s: _rng.normal(s) * 0.8)(B, Sq, D)),
            "k_cache": _w((lambda *s: _rng.normal(s) * 0.8)(B, Hkv, Sk, Dh)),
            "v_cache": _w((lambda *s: _rng.normal(s) * 0.05)(B, Hkv, Sk, Dh)),
            "wq": _w((lambda *s: _rng.normal(s) * 0.8)(D, Hq * Dh) * (D ** -0.5)),
            "wo": _w((lambda *s: _rng.normal(s) * 0.05)(Hq * Dh, D) * ((Hq * Dh) ** -0.5)),
        }
    _A_in = _A_setup()

    def _B_setup():
        B, Sq, D = 8, 240, 640
        Hq, Hkv, Sk, Dh = 32, 32, 1024, 192
        assert Hq % Hkv == 0, (Hq, Hkv)
        return {
            "x": _w((lambda *s: _rng.normal(s) * 0.8)(B, Sq, D)),
            "k_cache": _w((lambda *s: _rng.normal(s) * 0.8)(B, Hkv, Sk, Dh)),
            "v_cache": _w((lambda *s: _rng.normal(s) * 0.05)(B, Hkv, Sk, Dh)),
            "wq": _w((lambda *s: _rng.normal(s) * 0.8)(D, Hq * Dh) * (D ** -0.5)),
            "wo": _w((lambda *s: _rng.normal(s) * 0.05)(Hq * Dh, D) * ((Hq * Dh) ** -0.5)),
        }
    _B_in = _B_setup()

    return {
        "A_x": _A_in["x"],
        "A_k_cache": _A_in["k_cache"],
        "A_v_cache": _A_in["v_cache"],
        "A_wq": _A_in["wq"],
        "A_wo": _A_in["wo"],
        "B_x": _B_in["x"],
        "B_k_cache": _B_in["k_cache"],
        "B_v_cache": _B_in["v_cache"],
        "B_wq": _B_in["wq"],
        "B_wo": _B_in["wo"],
    }

def reference(A_x, A_k_cache, A_v_cache, A_wq, A_wo, B_x, B_k_cache, B_v_cache, B_wq, B_wo):
    def _A_ref(x, k_cache, v_cache, wq, wo):
        B, Sq, D = x.shape
        Hq, Dh = 32, 192
        Hkv = k_cache.shape[1]
        rep = Hq // Hkv
        q = (lambda x, *d: x.transpose(*d))((x @ wq).reshape(B, Sq, Hq, Dh), 0, 2, 1, 3)
        k = jnp.repeat(k_cache, rep, axis=1)
        v = jnp.repeat(v_cache, rep, axis=1)
        scores = jnp.einsum("bhqd,bhkd->bhqk", q, k) * (Dh ** -0.5)
        p = _softmax(scores, axis=-1)
        o = jnp.einsum("bhqk,bhkd->bhqd", p, v)
        return (lambda x, *d: x.transpose(*d))(o, 0, 2, 1, 3).reshape(B, Sq, Hq * Dh) @ wo

    def _B_ref(x, k_cache, v_cache, wq, wo):
        B, Sq, D = x.shape
        Hq, Dh = 32, 192
        Hkv = k_cache.shape[1]
        rep = Hq // Hkv
        q = (lambda x, *d: x.transpose(*d))((x @ wq).reshape(B, Sq, Hq, Dh), 0, 2, 1, 3)
        k = jnp.repeat(k_cache, rep, axis=1)
        v = jnp.repeat(v_cache, rep, axis=1)
        scores = jnp.einsum("bhqd,bhkd->bhqk", q, k) * (Dh ** -0.5)
        p = _softmax(scores, axis=-1)
        o = jnp.einsum("bhqk,bhkd->bhqd", p, v)
        return (lambda x, *d: x.transpose(*d))(o, 0, 2, 1, 3).reshape(B, Sq, Hq * Dh) @ wo

    a = _A_ref(A_x, A_k_cache, A_v_cache, A_wq, A_wo)
    b = _B_ref(B_x, B_k_cache, B_v_cache, B_wq, B_wo)
    return jnp.concatenate([a, b], axis=-1)
```

```python
import jax
import jax.numpy as jnp
from jax import lax
import jax.experimental.pallas as pl
import jax.experimental.pallas.tpu as pltpu

B, SQ, D = 8, 240, 640
H, SK, DH = 32, 1024, 192
LOG2E = 1.4426950408889634
NT = (((1,), (1,)), ((), ()))
NH = 4


def _schedule(n):
    P = n // 2
    s = [("Q", 0), ("QK", 0)]
    for p in range(P):
        s.append(("QK", 2 * p + 1))
        if p + 1 < P:
            s.append(("Q", p + 1))
        s.append(("PV", 2 * p))
        if p + 1 < P:
            if p > 0:
                s.append(("O", p - 1))
            s.append(("PV", 2 * p + 1))
            s.append(("QK", 2 * p + 2))
        else:
            s.append(("PV", 2 * p + 1))
            if p > 0:
                s.append(("O", p - 1))
    s.append(("O", P - 1))
    return s


def _kernel(xa, ka, va, wqa, woa, xb, kb, vb, wqb, wob, out_ref, acc_ref):
    hg = pl.program_id(0)
    b = pl.program_id(1)
    scale = (DH ** -0.5) * LOG2E
    refs = ((xa, ka, va, wqa, woa), (xb, kb, vb, wqb, wob))
    ppb = NH // 2
    xs = [xa[0], xb[0]]
    qps, ps, ls, ots, parts = {}, {}, {}, {}, {0: None, 1: None}
    done = {0: 0, 1: 0}
    for op, i in _schedule(2 * NH):
        if op == "Q":
            br, hp = divmod(i, ppb)
            qp = jnp.dot(xs[br], refs[br][3][:, hp * 2 * DH:(hp + 1) * 2 * DH],
                         preferred_element_type=jnp.float32)
            qps[i] = (qp * scale).astype(jnp.bfloat16)
        elif op == "QK":
            br, h = divmod(i, NH)
            j = i % 2
            q = qps[i // 2][:, j * DH:(j + 1) * DH]
            s = jnp.dot(q, refs[br][1][0, h], preferred_element_type=jnp.float32)
            m = jnp.max(s, axis=-1, keepdims=True)
            p = jnp.exp2(s - m)
            ls[i] = jnp.sum(p, axis=-1, keepdims=True)
            ps[i] = p.astype(jnp.bfloat16)
        elif op == "PV":
            br, h = divmod(i, NH)
            ots[i] = lax.dot_general(refs[br][2][0, h], ps[i], NT,
                                     preferred_element_type=jnp.float32)
        elif op == "O":
            br, hp = divmod(i, ppb)
            o = jnp.concatenate([ots[2 * i], ots[2 * i + 1]], axis=0).T
            lane = lax.broadcasted_iota(jnp.int32, (SQ, 2 * DH), 1)
            inv = jnp.where(lane < DH, 1.0 / ls[2 * i], 1.0 / ls[2 * i + 1])
            o = (o * inv).astype(jnp.bfloat16)
            pp = jnp.dot(o, refs[br][4][hp * 2 * DH:(hp + 1) * 2 * DH, :],
                         preferred_element_type=jnp.float32)
            if parts[br] is None:
                prev = jnp.where(hg == 0, 0.0, acc_ref[b, :, br * D:(br + 1) * D])
                parts[br] = prev + pp
            else:
                parts[br] = parts[br] + pp
            done[br] += 1
            if done[br] == ppb:
                tot = parts[br]
                acc_ref[b, :, br * D:(br + 1) * D] = tot
                out_ref[0, :, br * D:(br + 1) * D] = tot.astype(out_ref.dtype)


@jax.jit
def pallas_concat_heads__gqa_block_cached__gqa_block_cached__near_ridge_kernel(
    A_x: jax.Array,
    A_k_cache: jax.Array,
    A_v_cache: jax.Array,
    A_wq: jax.Array,
    A_wo: jax.Array,
    B_x: jax.Array,
    B_k_cache: jax.Array,
    B_v_cache: jax.Array,
    B_wq: jax.Array,
    B_wo: jax.Array,
):
    nhg = H // NH
    tr = lambda a: jnp.swapaxes(a, 2, 3)
    x_spec = pl.BlockSpec((1, SQ, D), lambda hg, b: (b, 0, 0))
    kv_spec = pl.BlockSpec((1, NH, DH, SK), lambda hg, b: (b, hg, 0, 0))
    wq_spec = pl.BlockSpec((D, NH * DH), lambda hg, b: (0, hg))
    wo_spec = pl.BlockSpec((NH * DH, D), lambda hg, b: (hg, 0))
    specs = [x_spec, kv_spec, kv_spec, wq_spec, wo_spec]
    return pl.pallas_call(
        _kernel,
        grid=(nhg, B),
        in_specs=specs + specs,
        out_specs=pl.BlockSpec(
            (1, SQ, 2 * D), lambda hg, b: (jnp.where(hg == nhg - 1, b, 0), 0, 0)),
        out_shape=jax.ShapeDtypeStruct((B, SQ, 2 * D), jnp.bfloat16),
        scratch_shapes=[pltpu.VMEM((B, SQ, 2 * D), jnp.float32)],
        compiler_params=pltpu.CompilerParams(
            dimension_semantics=("arbitrary", "arbitrary"),
            vmem_limit_bytes=100 * 1024 * 1024),
    )(A_x, tr(A_k_cache), tr(A_v_cache), A_wq, A_wo,
      B_x, tr(B_k_cache), tr(B_v_cache), B_wq, B_wo)
```

```python
import jax
import jax.numpy as jnp
from jax import lax
import jax.experimental.pallas as pl
import jax.experimental.pallas.tpu as pltpu

B, SQ, D = 8, 240, 640
H, SK, DH = 32, 1024, 192
NH = 4
NHG = H // NH
T = NHG * B
PW = 2 * DH
PPB = NH // 2
W2 = NH * DH
QR = D // B
OR = W2 // B
LOG2E = 1.4426950408889634
NT_DIMS = (((1,), (1,)), ((), ()))

LOOP_ORDER = ("Q0 QK0 QK1 Q1 PV0 QK2 PV1 PV2 Q2 QK3 O0 PV3 "
              "QK4 QK5 Q3 PV4 O1 QK6 PV5 QK7 PV6 PV7 O2 O3")
PEEL_ORDER = ("Q0 QK0 QK1 Q1 PV0 PV1 QK2 QK3 Q2 PV2 O0 PV3 "
              "QK4 QK5 Q3 PV4 PV5 QK6 O1 QK7 PV6 PV7 O2 O3")
PEEL_WAITS = ((0, 1, 3, 6, 8, 10, 12, 15, 17, 20), (0, 8, 16))


def _parse(order):
    ops = []
    for tok in order.split():
        name = tok.rstrip("0123456789")
        ops.append((name, int(tok[len(name):])))
    return ops


def _peel_plan(step, ops, wait_at):
    keys, waits = [], {}
    for pos, (op, i) in enumerate(ops):
        need = []
        if op == "Q":
            br, hp = divmod(i, PPB)
            if hp == 0:
                need.append(("x", br, 0))
            if step == 0:
                need.append(("wq", br, hp))
        elif op == "QK":
            need.append(("k",) + divmod(i, NH))
        elif op == "PV":
            need.append(("v",) + divmod(i, NH))
        elif step == 0:
            need.append(("wo",) + divmod(i, PPB))
        for key in need:
            keys.append(key)
            waits.setdefault(max(w for w in wait_at if w <= pos), []).append(key)
    return keys, waits


_LOOP_OPS = _parse(LOOP_ORDER)
_PEEL_OPS = _parse(PEEL_ORDER)
_PLANS = [_peel_plan(t, _PEEL_OPS, w) for t, w in enumerate(PEEL_WAITS)]
NPEEL = len(_PLANS)
NFINE = sum(len(k) for k, _ in _PLANS)


def _kernel(xa, ka, va, wqa, woa, xb, kb, vb, wqb, wob, out_hbm,
            xbuf, kvbuf, wqbuf, wobuf, acc_ref, obuf,
            xsem, kvsem, wqsem, wosem, osem, psem):
    hbm = ((xa, ka, va, wqa, woa), (xb, kb, vb, wqb, wob))
    scale = (DH ** -0.5) * LOG2E
    cp = pltpu.make_async_copy

    def step_start(t, slot):
        hg, b = t >> 3, t & (B - 1)
        for br in range(2):
            cp(hbm[br][0].at[b], xbuf.at[slot, br], xsem.at[slot]).start()
            for kv in range(2):
                cp(hbm[br][1 + kv].at[b, pl.ds(hg * NH, NH)],
                   kvbuf.at[slot, kv, br], kvsem.at[slot]).start()

    def step_wait(slot):
        cp(xbuf.at[slot], xbuf.at[slot], xsem.at[slot]).wait()
        cp(kvbuf.at[slot], kvbuf.at[slot], kvsem.at[slot]).wait()

    def w_slice_start(hg, slot, j):
        col = pl.multiple_of(hg * W2, 128)
        qr = pl.multiple_of(j * QR, 16)
        orr = pl.multiple_of(j * OR, 16)
        for br in range(2):
            cp(hbm[br][3].at[pl.ds(qr, QR), pl.ds(col, W2)],
               wqbuf.at[slot, br, pl.ds(qr, QR)], wqsem.at[slot]).start()
            cp(hbm[br][4].at[pl.ds(col + orr, OR), :],
               wobuf.at[slot, br, pl.ds(orr, OR)], wosem.at[slot]).start()

    def w_wait(slot):
        cp(wqbuf.at[slot], wqbuf.at[slot], wqsem.at[slot]).wait()
        cp(wobuf.at[slot], wobuf.at[slot], wosem.at[slot]).wait()

    def fine_copy(key, t, sem):
        kind, br, j = key
        if kind == "x":
            return cp(hbm[br][0].at[t], xbuf.at[t & 1, br], sem)
        if kind in ("k", "v"):
            kv = 0 if kind == "k" else 1
            return cp(hbm[br][1 + kv].at[t, j], kvbuf.at[t & 1, kv, br, j], sem)
        if kind == "wq":
            return cp(hbm[br][3].at[:, pl.ds(j * PW, PW)],
                      wqbuf.at[0, br, :, pl.ds(j * PW, PW)], sem)
        return cp(hbm[br][4].at[pl.ds(j * PW, PW), :],
                  wobuf.at[0, br, pl.ds(j * PW, PW), :], sem)

    def out_copy(b):
        return cp(obuf.at[b], out_hbm.at[b], osem.at[b])

    def compute(ops, hg, b, slot, wslot, hooks):
        qs, ps, ls, ots, parts, done = {}, {}, {}, {}, {}, {}
        for pos, (op, i) in enumerate(ops):
            if pos in hooks:
                hooks[pos]()
            if op == "Q":
                br, hp = divmod(i, PPB)
                q = jnp.dot(xbuf[slot, br], wqbuf[wslot, br, :, hp * PW:(hp + 1) * PW],
                            preferred_element_type=jnp.float32)
                qs[i] = (q * scale).astype(jnp.bfloat16)
            elif op == "QK":
                br, h = divmod(i, NH)
                j = i % 2
                s = jnp.dot(qs[i // 2][:, j * DH:(j + 1) * DH], kvbuf[slot, 0, br, h],
                            preferred_element_type=jnp.float32)
                m = jnp.max(s, axis=-1, keepdims=True)
                p = jnp.exp2(s - m)
                ls[i] = jnp.sum(p, axis=-1, keepdims=True)
                ps[i] = p.astype(jnp.bfloat16)
            elif op == "PV":
                br, h = divmod(i, NH)
                ots[i] = lax.dot_general(kvbuf[slot, 1, br, h], ps[i], NT_DIMS,
                                         preferred_element_type=jnp.float32)
            else:
                br, hp = divmod(i, PPB)
                o = jnp.concatenate([ots[2 * i], ots[2 * i + 1]], axis=0).T
                lane = lax.broadcasted_iota(jnp.int32, (SQ, PW), 1)
                inv = jnp.where(lane < DH, 1.0 / ls[2 * i], 1.0 / ls[2 * i + 1])
                o = (o * inv).astype(jnp.bfloat16)
                part = jnp.dot(o, wobuf[wslot, br, hp * PW:(hp + 1) * PW, :],
                               preferred_element_type=jnp.float32)
                cols = slice(br * D, (br + 1) * D)
                if br in parts:
                    parts[br] = parts[br] + part
                elif isinstance(hg, int):
                    parts[br], done[br] = part, 0
                else:
                    prev = jnp.where(hg == 0, 0.0, acc_ref[b, :, cols])
                    parts[br], done[br] = prev + part, 0
                done[br] += 1
                if done[br] == PPB:
                    acc_ref[b, :, cols] = parts[br]
                    obuf[b, :, cols] = parts[br].astype(obuf.dtype)

    copies, base = [], 0
    for t, (keys, _) in enumerate(_PLANS):
        copies.append({k: fine_copy(k, t, psem.at[base + j]) for j, k in enumerate(keys)})
        base += len(keys)
    for k in _PLANS[0][0]:
        copies[0][k].start()

    for t, (_, waits) in enumerate(_PLANS):
        def hook(pos, t=t, waits=waits):
            if pos == 0:
                if t + 1 < NPEEL:
                    for k in _PLANS[t + 1][0]:
                        copies[t + 1][k].start()
                else:
                    step_start(t + 1, (t + 1) & 1)
                    for j in range(NPEEL):
                        w_slice_start(1, 1, j)
            for k in waits.get(pos, ()):
                copies[t][k].wait()
        compute(_PEEL_OPS, 0, t, t & 1, 0,
                {pos: (lambda pos=pos: hook(pos)) for pos in set(waits) | {0}})
    step_wait(NPEEL & 1)

    def body(t, carry):
        hg, b = t >> 3, t & (B - 1)
        slot, wslot = t & 1, hg & 1

        @pl.when(b == 0)
        def _():
            w_wait(wslot)

        step_start(jnp.minimum(t + 1, T - 1), 1 - slot)

        def next_weights():
            w_slice_start(jnp.minimum(hg + 1, NHG - 1), 1 - wslot, b)

        compute(_LOOP_OPS, hg, b, slot, wslot, {2: next_weights})

        @pl.when(hg == NHG - 1)
        def _():
            out_copy(b).start()

        step_wait(1 - slot)
        return carry

    lax.fori_loop(NPEEL, T, body, 0)
    w_wait(NHG & 1)
    for b in range(B):
        out_copy(b).wait()


@jax.jit
def pallas_concat_heads__gqa_block_cached__gqa_block_cached__near_ridge_kernel(
    A_x: jax.Array,
    A_k_cache: jax.Array,
    A_v_cache: jax.Array,
    A_wq: jax.Array,
    A_wo: jax.Array,
    B_x: jax.Array,
    B_k_cache: jax.Array,
    B_v_cache: jax.Array,
    B_wq: jax.Array,
    B_wo: jax.Array,
):
    tr = lambda a: jnp.swapaxes(a, 2, 3)
    any_spec = pl.BlockSpec(memory_space=pl.ANY)
    return pl.pallas_call(
        _kernel,
        in_specs=[any_spec] * 10,
        out_specs=any_spec,
        out_shape=jax.ShapeDtypeStruct((B, SQ, 2 * D), jnp.bfloat16),
        scratch_shapes=[
            pltpu.VMEM((2, 2, SQ, D), jnp.bfloat16),
            pltpu.VMEM((2, 2, 2, NH, DH, SK), jnp.bfloat16),
            pltpu.VMEM((2, 2, D, W2), jnp.bfloat16),
            pltpu.VMEM((2, 2, W2, D), jnp.bfloat16),
            pltpu.VMEM((B, SQ, 2 * D), jnp.float32),
            pltpu.VMEM((B, SQ, 2 * D), jnp.bfloat16),
            pltpu.SemaphoreType.DMA((2,)),
            pltpu.SemaphoreType.DMA((2,)),
            pltpu.SemaphoreType.DMA((2,)),
            pltpu.SemaphoreType.DMA((2,)),
            pltpu.SemaphoreType.DMA((B,)),
            pltpu.SemaphoreType.DMA((NFINE,)),
        ],
        compiler_params=pltpu.CompilerParams(vmem_limit_bytes=100 * 1024 * 1024),
    )(A_x, tr(A_k_cache), tr(A_v_cache), A_wq, A_wo,
      B_x, tr(B_k_cache), tr(B_v_cache), B_wq, B_wo)
```

```python
import jax
import jax.numpy as jnp
from jax import lax
import jax.experimental.pallas as pl
import jax.experimental.pallas.tpu as pltpu

B, SQ, D = 8, 240, 640
H, SK, DH = 32, 1024, 192
NH = 4
NHG = H // NH
T = NHG * B
PW = 2 * DH
PPB = NH // 2
W2 = NH * DH
QR = D // B
OR = W2 // B
LOG2E = 1.4426950408889634
NT_DIMS = (((1,), (1,)), ((), ()))

LOOP_ORDER = ("Q0 QK0 QK1 Q1 PV0 QK2 PV1 PV2 Q2 QK3 O0 PV3 "
              "QK4 QK5 Q3 PV4 O1 QK6 PV5 QK7 PV6 PV7 O2 O3")
PEEL_ORDERS = (("Q0 QK0 QK1 Q1 PV0 PV1 QK2 QK3 Q2 PV2 O0 PV3 "
                "QK4 QK5 Q3 PV4 PV5 QK6 O1 QK7 PV6 PV7 O2 O3"),
               ("Q0 QK0 QK1 Q1 PV0 PV1 QK2 QK3 Q2 PV2 O0 QK4 "
                "PV3 QK5 Q3 O1 PV4 PV5 QK6 QK7 O2 PV6 PV7 O3"))
PEEL_WAITS = ((0, 1, 3, 6, 9, 12, 15, 17, 21), (0, 4, 16))
W_PREFETCH_POS = 2
OUT_A_POS = 20


def _parse(order):
    ops = []
    for tok in order.split():
        name = tok.rstrip("0123456789")
        ops.append((name, int(tok[len(name):])))
    return ops


def _peel_plan(step, ops, wait_at):
    keys, waits = [], {}
    for pos, (op, i) in enumerate(ops):
        need = []
        if op == "Q":
            br, hp = divmod(i, PPB)
            if hp == 0:
                need.append(("x", br, 0))
            if step == 0:
                need.append(("wq", br, hp))
        elif op == "QK":
            need.append(("k",) + divmod(i, NH))
        elif op == "PV":
            need.append(("v",) + divmod(i, NH))
        elif step == 0:
            need.append(("wo",) + divmod(i, PPB))
        for key in need:
            keys.append(key)
            waits.setdefault(max(w for w in wait_at if w <= pos), []).append(key)
    return keys, waits


_LOOP_OPS = _parse(LOOP_ORDER)
_PEEL_OPS = [_parse(o) for o in PEEL_ORDERS]
_PLANS = [_peel_plan(t, _PEEL_OPS[t], w) for t, w in enumerate(PEEL_WAITS)]
NPEEL = len(_PLANS)
NFINE = sum(len(k) for k, _ in _PLANS)


def _kernel(xa, ka, va, wqa, woa, xb, kb, vb, wqb, wob, out_hbm,
            xbuf, kvbuf, wqbuf, wobuf, acc_ref, obuf,
            xsem, kvsem, wqsem, wosem, osem, psem):
    hbm = ((xa, ka, va, wqa, woa), (xb, kb, vb, wqb, wob))
    scale = (DH ** -0.5) * LOG2E
    cp = pltpu.make_async_copy

    def step_start(t, slot):
        hg, b = t >> 3, t & (B - 1)
        for br in range(2):
            cp(hbm[br][0].at[b], xbuf.at[slot, br], xsem.at[slot]).start()
            for kv in range(2):
                cp(hbm[br][1 + kv].at[b, pl.ds(hg * NH, NH)],
                   kvbuf.at[slot, kv, br], kvsem.at[slot]).start()

    def step_wait(slot):
        cp(xbuf.at[slot], xbuf.at[slot], xsem.at[slot]).wait()
        cp(kvbuf.at[slot], kvbuf.at[slot], kvsem.at[slot]).wait()

    def w_slice_start(hg, slot, j):
        col = pl.multiple_of(hg * W2, 128)
        qr = pl.multiple_of(j * QR, 16)
        orr = pl.multiple_of(j * OR, 16)
        for br in range(2):
            cp(hbm[br][3].at[pl.ds(qr, QR), pl.ds(col, W2)],
               wqbuf.at[slot, br, pl.ds(qr, QR)], wqsem.at[slot]).start()
            cp(hbm[br][4].at[pl.ds(col + orr, OR), :],
               wobuf.at[slot, br, pl.ds(orr, OR)], wosem.at[slot]).start()

    def w_wait(slot):
        cp(wqbuf.at[slot], wqbuf.at[slot], wqsem.at[slot]).wait()
        cp(wobuf.at[slot], wobuf.at[slot], wosem.at[slot]).wait()

    def fine_copy(key, t, sem):
        kind, br, j = key
        if kind == "x":
            return cp(hbm[br][0].at[t], xbuf.at[t & 1, br], sem)
        if kind in ("k", "v"):
            kv = 0 if kind == "k" else 1
            return cp(hbm[br][1 + kv].at[t, j], kvbuf.at[t & 1, kv, br, j], sem)
        if kind == "wq":
            return cp(hbm[br][3].at[:, pl.ds(j * PW, PW)],
                      wqbuf.at[0, br, :, pl.ds(j * PW, PW)], sem)
        return cp(hbm[br][4].at[pl.ds(j * PW, PW), :],
                  wobuf.at[0, br, pl.ds(j * PW, PW), :], sem)

    def out_copy(b, br):
        cols = pl.ds(br * D, D)
        return cp(obuf.at[b, :, cols], out_hbm.at[b, :, cols], osem.at[br, b])

    def compute(ops, hg, b, slot, wslot, hooks):
        qs, ps, ls, ots, parts, done = {}, {}, {}, {}, {}, {}
        for pos, (op, i) in enumerate(ops):
            if pos in hooks:
                hooks[pos]()
            if op == "Q":
                br, hp = divmod(i, PPB)
                q = jnp.dot(xbuf[slot, br], wqbuf[wslot, br, :, hp * PW:(hp + 1) * PW],
                            preferred_element_type=jnp.float32)
                qs[i] = (q * scale).astype(jnp.bfloat16)
            elif op == "QK":
                br, h = divmod(i, NH)
                j = i % 2
                s = jnp.dot(qs[i // 2][:, j * DH:(j + 1) * DH], kvbuf[slot, 0, br, h],
                            preferred_element_type=jnp.float32)
                m = jnp.max(s, axis=-1, keepdims=True)
                p = jnp.exp2(s - m)
                ls[i] = jnp.sum(p, axis=-1, keepdims=True)
                ps[i] = p.astype(jnp.bfloat16)
            elif op == "PV":
                br, h = divmod(i, NH)
                ots[i] = lax.dot_general(kvbuf[slot, 1, br, h], ps[i], NT_DIMS,
                                         preferred_element_type=jnp.float32)
            else:
                br, hp = divmod(i, PPB)
                o = jnp.concatenate([ots[2 * i], ots[2 * i + 1]], axis=0).T
                lane = lax.broadcasted_iota(jnp.int32, (SQ, PW), 1)
                inv = jnp.where(lane < DH, 1.0 / ls[2 * i], 1.0 / ls[2 * i + 1])
                o = (o * inv).astype(jnp.bfloat16)
                part = jnp.dot(o, wobuf[wslot, br, hp * PW:(hp + 1) * PW, :],
                               preferred_element_type=jnp.float32)
                cols = slice(br * D, (br + 1) * D)
                if br in parts:
                    parts[br] = parts[br] + part
                elif isinstance(hg, int):
                    parts[br], done[br] = part, 0
                else:
                    prev = jnp.where(hg == 0, 0.0, acc_ref[b, :, cols])
                    parts[br], done[br] = prev + part, 0
                done[br] += 1
                if done[br] == PPB:
                    acc_ref[b, :, cols] = parts[br]
                    obuf[b, :, cols] = parts[br].astype(obuf.dtype)

    copies, base = [], 0
    for t, (keys, _) in enumerate(_PLANS):
        copies.append({k: fine_copy(k, t, psem.at[base + j]) for j, k in enumerate(keys)})
        base += len(keys)
    for k in _PLANS[0][0]:
        copies[0][k].start()

    for t, (_, waits) in enumerate(_PLANS):
        def hook(pos, t=t, waits=waits):
            if pos == 0:
                if t + 1 < NPEEL:
                    for k in _PLANS[t + 1][0]:
                        copies[t + 1][k].start()
                else:
                    step_start(t + 1, (t + 1) & 1)
                    for j in range(NPEEL):
                        w_slice_start(1, 1, j)
            for k in waits.get(pos, ()):
                copies[t][k].wait()
        compute(_PEEL_OPS[t], 0, t, t & 1, 0,
                {pos: (lambda pos=pos: hook(pos)) for pos in sorted(waits)})
    step_wait(NPEEL & 1)

    def body(t, carry):
        hg, b = t >> 3, t & (B - 1)
        slot, wslot = t & 1, hg & 1

        step_start(jnp.minimum(t + 1, T - 1), 1 - slot)

        def next_weights():
            w_slice_start(jnp.minimum(hg + 1, NHG - 1), 1 - wslot, b)

        def write_out(br):
            @pl.when(hg == NHG - 1)
            def _():
                out_copy(b, br).start()

        compute(_LOOP_OPS, hg, b, slot, wslot,
                {W_PREFETCH_POS: next_weights, OUT_A_POS: lambda: write_out(0)})
        write_out(1)

        @pl.when(b == B - 1)
        def _():
            w_wait(1 - wslot)

        step_wait(1 - slot)
        return carry

    lax.fori_loop(NPEEL, T, body, 0)
    for b in range(B):
        for br in range(2):
            out_copy(b, br).wait()


@jax.jit
def pallas_concat_heads__gqa_block_cached__gqa_block_cached__near_ridge_kernel(
    A_x: jax.Array,
    A_k_cache: jax.Array,
    A_v_cache: jax.Array,
    A_wq: jax.Array,
    A_wo: jax.Array,
    B_x: jax.Array,
    B_k_cache: jax.Array,
    B_v_cache: jax.Array,
    B_wq: jax.Array,
    B_wo: jax.Array,
):
    tr = lambda a: jnp.swapaxes(a, 2, 3)
    any_spec = pl.BlockSpec(memory_space=pl.ANY)
    return pl.pallas_call(
        _kernel,
        in_specs=[any_spec] * 10,
        out_specs=any_spec,
        out_shape=jax.ShapeDtypeStruct((B, SQ, 2 * D), jnp.bfloat16),
        scratch_shapes=[
            pltpu.VMEM((2, 2, SQ, D), jnp.bfloat16),
            pltpu.VMEM((2, 2, 2, NH, DH, SK), jnp.bfloat16),
            pltpu.VMEM((2, 2, D, W2), jnp.bfloat16),
            pltpu.VMEM((2, 2, W2, D), jnp.bfloat16),
            pltpu.VMEM((B, SQ, 2 * D), jnp.float32),
            pltpu.VMEM((B, SQ, 2 * D), jnp.bfloat16),
            pltpu.SemaphoreType.DMA((2,)),
            pltpu.SemaphoreType.DMA((2,)),
            pltpu.SemaphoreType.DMA((2,)),
            pltpu.SemaphoreType.DMA((2,)),
            pltpu.SemaphoreType.DMA((2, B)),
            pltpu.SemaphoreType.DMA((NFINE,)),
        ],
        compiler_params=pltpu.CompilerParams(vmem_limit_bytes=100 * 1024 * 1024),
    )(A_x, tr(A_k_cache), tr(A_v_cache), A_wq, A_wo,
      B_x, tr(B_k_cache), tr(B_v_cache), B_wq, B_wo)
```
